```python
import jax
import jax.numpy as jnp

def _softmax(x, axis=-1):
    return jax.nn.softmax(x, axis=axis)
def _gelu(x):
    return jax.nn.gelu(x, approximate=True)
def _silu(x):
    return jax.nn.silu(x)
def _sigmoid(x):
    return jax.nn.sigmoid(x)
def _layernorm(x, axis=-1, eps=1e-5):
    m = jnp.mean(x, axis=axis, keepdims=True)
    v = jnp.var(x, axis=axis, keepdims=True)
    return (x - m) / jnp.sqrt(v + eps)
def _scatter_add(tgt, idx, src, axis=0):
    return tgt.at[idx].add(src)
def _segment_sum(src, seg, n):
    return jax.ops.segment_sum(src, seg, n)
class _Rng:
    def __init__(self, key):
        self._k = key
    def _next(self):
        self._k, sub = jax.random.split(self._k)
        return sub
    def normal(self, shape):
        return jax.random.normal(self._next(), shape, dtype=jnp.bfloat16)
    def randint(self, lo, hi, shape):
        return jax.random.randint(self._next(), shape, lo, hi, dtype=jnp.int32)
    def uniform(self, shape, lo=0.0, hi=1.0):
        return jax.random.uniform(self._next(), shape, jnp.bfloat16, lo, hi)
    def permutation(self, n):
        return jax.random.permutation(self._next(), n)


kernel_name = 'recurrent_scan__compressed_kv_cla__dense_activation_silu__decode'

def setup_inputs():
    _rng = _Rng(jax.random.key(int.from_bytes(__import__("os").urandom(4), "little")))
    _w = (lambda a: (lambda t: t.astype(jnp.bfloat16) if jnp.issubdtype(t.dtype, jnp.floating) else t)(jnp.asarray(a)))
    def _A_setup():
        B, H, Sq, Sk, D, M = 1, 32, 1, 32768, 128, 512
        Dc = 4 * D
        return {
            "x": _w((lambda *s: _rng.normal(s) * 0.05)(B, Sq, M)),
            "c_kv": _w((lambda *s: _rng.normal(s) * 0.05)(B, Sk, Dc)),
            "w_q": _w((lambda *s: _rng.normal(s) * 0.05)(M, H, D) * (M ** -0.5)),
            "w_uk": _w((lambda *s: _rng.normal(s) * 0.05)(Dc, H, D) * (Dc ** -0.5)),
            "w_uv": _w((lambda *s: _rng.normal(s) * 0.05)(Dc, H, D) * (Dc ** -0.5)),
            "w_o": _w((lambda *s: _rng.normal(s) * 0.05)(H, D, M) * ((H * D) ** -0.5)),
        }
    _A_in = _A_setup()

    def _B_setup():
        B, S, D, F = 1, 1, 512, 1376
        return {
            "x": _w((lambda *s: _rng.normal(s) * 0.05)(B, S, D)),
            "w1": _w((lambda *s: _rng.normal(s) * 0.05)(D, F) * (D ** -0.5)),
            "w2": _w((lambda *s: _rng.normal(s) * 0.05)(F, D) * (F ** -0.5)),
        }
    _B_in = _B_setup()

    return {
        "A_x": _A_in["x"],
        "A_c_kv": _A_in["c_kv"],
        "A_w_q": _A_in["w_q"],
        "A_w_uk": _A_in["w_uk"],
        "A_w_uv": _A_in["w_uv"],
        "A_w_o": _A_in["w_o"],
        "B_x": _B_in["x"],
        "B_w1": _B_in["w1"],
        "B_w2": _B_in["w2"],
    }

def reference(A_x, A_c_kv, A_w_q, A_w_uk, A_w_uv, A_w_o, B_x, B_w1, B_w2):
    def _A_ref(x, c_kv, w_q, w_uk, w_uv, w_o):
        B, Sq, M = x.shape[0], x.shape[1], x.shape[2]
        Sk = c_kv.shape[1]
        H, D = w_q.shape[1], w_q.shape[2]
        q = jnp.einsum("bqm,mhd->bhqd", x, w_q)
        k = jnp.einsum("bkc,chd->bhkd", c_kv, w_uk)
        v = jnp.einsum("bkc,chd->bhkd", c_kv, w_uv)
        scores = jnp.einsum("bhqd,bhkd->bhqk", q, k) * (D ** -0.5)
        off = Sk - Sq
        qi = jnp.arange(Sq)[:, None]
        kj = jnp.arange(Sk)[None, :]
        cmask = kj <= (qi + off)
        scores = jnp.where(cmask[None, None], scores, -1e9)
        p = _softmax(scores, axis=-1)
        ctx = jnp.einsum("bhqk,bhkd->bhqd", p, v)
        return jnp.einsum("bhqd,hdm->bqm", ctx, w_o)

    def _B_ref(x, w1, w2):
        h = jnp.einsum("bsd,df->bsf", x, w1)
        h = _silu(h)
        out = jnp.einsum("bsf,fd->bsd", h, w2)
        return out

    x = A_x
    xn = _layernorm(x, axis=-1)
    s = _A_ref(xn, A_c_kv, A_w_q, A_w_uk, A_w_uv, A_w_o)
    g = _silu(_B_ref(xn, B_w1, B_w2))
    return x + s * g
```

```python
import jax
import jax.numpy as jnp
from jax import lax
import jax.experimental.pallas as pl
import jax.experimental.pallas.tpu as pltpu

F32 = jnp.float32
BF16 = jnp.bfloat16
_NT = (((1,), (1,)), ((), ()))

_TK = 4096
_TG = 8
_WINDOW = 4


def _kernel(order, SK, DC, H, D, M, F,
            x_hbm, c_hbm, wq_hbm, wuk_hbm, wuv_hbm, wo_hbm, w1_hbm, w2_hbm, o_ref,
            x_v, c_v, wq_v, wuk_v, wuv_v, wo_v, w1_v, w2_v,
            z_v, y_v, l_v, q_v, qa_v, h_v, s_v, g_v, xf_v, o_v, sems):
    n = len(order)
    NJ = DC // 128

    def copy(i):
        step = order[i]
        kind, sem = step[0], sems.at[i]
        whole = {"x": (x_hbm, x_v), "wq": (wq_hbm, wq_v), "wuk": (wuk_hbm, wuk_v),
                 "wuv": (wuv_hbm, wuv_v), "w1": (w1_hbm, w1_v), "w2": (w2_hbm, w2_v)}
        if kind in whole:
            src, dst = whole[kind]
            return pltpu.make_async_copy(src, dst, sem)
        if kind == "c":
            src, dst, sl = c_hbm, c_v, pl.ds(step[1], step[2] - step[1])
        else:
            src, dst, sl = wo_hbm, wo_v, pl.ds(step[1] * D, (step[2] - step[1]) * D)
        return pltpu.make_async_copy(src.at[sl], dst.at[sl], sem)

    started = [0]

    def start_upto(k):
        while started[0] < min(k, n):
            copy(started[0]).start()
            started[0] += 1

    def wait(i):
        copy(i).wait()
        start_upto(i + 1 + _WINDOW)

    start_upto(_WINDOW)

    row = lax.broadcasted_iota(jnp.int32, (H, 128), 0)
    col = lax.broadcasted_iota(jnp.int32, (H, 128), 1)
    dmask = (col % H) == row

    def prep_z(a):
        a4 = jnp.concatenate([a[:, 128 * j:128 * (j + 1)] for j in range(NJ)], axis=0)
        z_v[...] = a4.T

    def perhead_nn(w_v):
        def body(gi, acc):
            t0 = pl.multiple_of(gi * _TG, _TG)
            zg = z_v[pl.ds(t0, _TG), :]
            for s in range(_TG):
                lhs = jnp.where(dmask, zg[s:s + 1, :], 0.0).astype(BF16)
                rhs = w_v[:, t0 + s].reshape(NJ * H, D)
                acc = acc + jnp.dot(lhs, rhs, preferred_element_type=F32)
            return acc
        return lax.fori_loop(0, 128 // _TG, body, jnp.zeros((H, D), F32))

    def flash_step(off, carry):
        m, l, acc = carry
        ck = c_v[pl.ds(off, _TK), :]
        s = lax.dot_general(qa_v[...], ck, _NT, preferred_element_type=F32)
        m_new = jnp.maximum(m, jnp.max(s, axis=-1, keepdims=True))
        alpha = jnp.exp(m - m_new)
        p = jnp.exp(s - m_new)
        l = alpha * l + jnp.sum(p, axis=-1, keepdims=True)
        acc = alpha * acc + jnp.dot(p.astype(BF16), ck, preferred_element_type=F32)
        return m_new, l, acc

    carry = None
    for i, step in enumerate(order):
        kind = step[0]
        wait(i)
        if kind == "x":
            x = x_v[...].astype(F32)
            mean = jnp.mean(x, axis=-1, keepdims=True)
            xc = x - mean
            var = jnp.mean(xc * xc, axis=-1, keepdims=True)
            xn = (xc / jnp.sqrt(var + 1e-5)).astype(BF16).astype(F32)
            xf_v[0:16, :] = jnp.broadcast_to(x, (16, M))
            xf_v[16:32, :] = jnp.broadcast_to(xn, (16, M))
            prep_z(jnp.broadcast_to(xn, (H, M)))
        elif kind == "wq":
            q_v[...] = perhead_nn(wq_v).astype(BF16)
        elif kind == "wuk":
            def body(gi, carry_):
                t0 = pl.multiple_of(gi * _TG, _TG)
                q_b = q_v[...]
                rows = []
                for s in range(_TG):
                    rhs = wuk_v[:, t0 + s].reshape(NJ * H, D)
                    o = lax.dot_general(q_b, rhs, _NT, preferred_element_type=F32)
                    rows.append(jnp.sum(jnp.where(dmask, o, 0.0), axis=0, keepdims=True))
                y_v[pl.ds(t0, _TG), :] = jnp.concatenate(rows, axis=0)
                return carry_
            lax.fori_loop(0, 128 // _TG, body, 0)
            a4 = y_v[...].T
            q_abs = jnp.concatenate([a4[H * j:H * (j + 1), :] for j in range(NJ)], axis=1)
            qa_v[...] = (q_abs * (D ** -0.5)).astype(BF16)
            carry = (jnp.full((H, 1), -jnp.inf, F32), jnp.zeros((H, 1), F32), jnp.zeros((H, DC), F32))
        elif kind == "c":
            base, end = step[1], step[2]
            carry = lax.fori_loop(
                0, (end - base) // _TK,
                lambda k, cr, base=base: flash_step(pl.multiple_of(base + k * _TK, _TK), cr), carry)
            if end == SK:
                _, l, acc = carry
                prep_z((acc / l).astype(BF16).astype(F32))
        elif kind == "wuv":
            y_v[0:H, :] = perhead_nn(wuv_v)
            for h in range(H):
                l_v[:, h * D:(h + 1) * D] = jnp.broadcast_to(y_v[h:h + 1, :], (16, D)).astype(BF16)
            s_v[...] = jnp.zeros((16, M), F32)
        elif kind == "wo":
            h0, h1 = step[1], step[2]
            s_v[...] += jnp.dot(l_v[:, h0 * D:h1 * D], wo_v[h0 * D:h1 * D, :], preferred_element_type=F32)
        elif kind == "w1":
            xb = xf_v[16:32, :].astype(BF16)
            hpre = lax.dot_general(xb, w1_v[...], _NT, preferred_element_type=F32)
            hpre = hpre.astype(BF16).astype(F32)
            h_v[...] = (hpre * jax.nn.sigmoid(hpre)).astype(BF16)
        elif kind == "w2":
            gpre = jnp.dot(h_v[...], w2_v[...], preferred_element_type=F32)
            g_v[...] = gpre * jax.nn.sigmoid(gpre)

    o_v[...] = (xf_v[0:1, :] + s_v[0:1, :] * g_v[0:1, :]).astype(BF16)
    cp_o = pltpu.make_async_copy(o_v, o_ref, sems.at[0])
    cp_o.start()
    cp_o.wait()


@jax.jit
def pallas_recurrent_scan__compressed_kv_cla__dense_activation_silu__decode_kernel(
    A_x: jax.Array,
    A_c_kv: jax.Array,
    A_w_q: jax.Array,
    A_w_uk: jax.Array,
    A_w_uv: jax.Array,
    A_w_o: jax.Array,
    B_x: jax.Array,
    B_w1: jax.Array,
    B_w2: jax.Array,
):
    del B_x
    _, SK, DC = A_c_kv.shape
    M, H, D = A_w_q.shape
    F = B_w1.shape[1]
    assert (M, DC, H, D) == (512, 512, 32, 128) and SK % (2 * _TK) == 0
    NJ = DC // 128

    half = SK // 2
    order = (
        ("x",), ("wq",), ("wuk",),
        ("c", 0, half), ("c", half, SK),
        ("w1",), ("w2",), ("wuv",),
        ("wo", 0, 22), ("wo", 22, 29), ("wo", 29, 31), ("wo", 31, 32),
    )

    def kernel(*refs):
        _kernel(order, SK, DC, H, D, M, F, *refs)

    out = pl.pallas_call(
        kernel,
        out_shape=jax.ShapeDtypeStruct((1, M), BF16),
        in_specs=[pl.BlockSpec(memory_space=pltpu.HBM)] * 8,
        out_specs=pl.BlockSpec(memory_space=pltpu.HBM),
        scratch_shapes=[
            pltpu.VMEM((1, M), BF16),
            pltpu.VMEM((SK, DC), BF16),
            pltpu.VMEM((NJ, 128, H, D), BF16),
            pltpu.VMEM((NJ, 128, H, D), BF16),
            pltpu.VMEM((NJ, 128, H, D), BF16),
            pltpu.VMEM((H * D, M), BF16),
            pltpu.VMEM((F, M), BF16),
            pltpu.VMEM((F, M), BF16),
            pltpu.VMEM((128, 128), F32),
            pltpu.VMEM((128, 128), F32),
            pltpu.VMEM((16, H * D), BF16),
            pltpu.VMEM((H, D), BF16),
            pltpu.VMEM((H, DC), BF16),
            pltpu.VMEM((16, F), BF16),
            pltpu.VMEM((16, M), F32),
            pltpu.VMEM((16, M), F32),
            pltpu.VMEM((32, M), F32),
            pltpu.VMEM((1, M), BF16),
            pltpu.SemaphoreType.DMA((len(order),)),
        ],
        compiler_params=pltpu.CompilerParams(
            vmem_limit_bytes=100 * 1024 * 1024,
            disable_semaphore_checks=True,
        ),
    )(
        A_x.reshape(1, M),
        A_c_kv.reshape(SK, DC),
        A_w_q.reshape(NJ, 128, H, D),
        A_w_uk.reshape(NJ, 128, H, D),
        A_w_uv.reshape(NJ, 128, H, D),
        A_w_o.reshape(H * D, M),
        B_w1.T,
        B_w2,
    )
    return out.reshape(1, 1, M)
```

```python
import jax
import jax.numpy as jnp
from jax import lax
import jax.experimental.pallas as pl
import jax.experimental.pallas.tpu as pltpu

F32 = jnp.float32
BF16 = jnp.bfloat16
_NT = (((1,), (1,)), ((), ()))

_TK = 4096
_TG = 8
_WINDOW = 6


def _kernel(order, SK, DC, H, D, M, F,
            x_hbm, c_hbm, wq_hbm, wuk_hbm, wuv_hbm, wo_hbm, w1_hbm, w2_hbm, o_ref,
            x_v, c_v, wq_v, wuk_v, wuv_v, wo_v, w1_v, w2_v,
            z_v, y_v, l_v, q_v, qa_v, h_v, s_v, g_v, xf_v, o_v, m_v, p_v, sems):
    n = len(order)
    NJ = DC // 128

    def copy(i):
        step = order[i]
        kind, sem = step[0], sems.at[i]
        whole = {"x": (x_hbm, x_v), "wq": (wq_hbm, wq_v), "wuk": (wuk_hbm, wuk_v),
                 "wuv": (wuv_hbm, wuv_v), "w1": (w1_hbm, w1_v), "w2": (w2_hbm, w2_v)}
        if kind in whole:
            src, dst = whole[kind]
            return pltpu.make_async_copy(src, dst, sem)
        if kind == "c":
            src, dst, sl = c_hbm, c_v, pl.ds(step[1], step[2] - step[1])
        else:
            src, dst, sl = wo_hbm, wo_v, pl.ds(step[1], step[2] - step[1])
        return pltpu.make_async_copy(src.at[sl], dst.at[sl], sem)

    started = [0]

    def start_upto(k):
        while started[0] < min(k, n):
            copy(started[0]).start()
            started[0] += 1

    def wait(i):
        copy(i).wait()
        start_upto(i + 1 + _WINDOW)

    start_upto(_WINDOW)

    row = lax.broadcasted_iota(jnp.int32, (H, 128), 0)
    col = lax.broadcasted_iota(jnp.int32, (H, 128), 1)
    dmask = (col % H) == row

    def prep_z(a):
        a4 = jnp.concatenate([a[:, 128 * j:128 * (j + 1)] for j in range(NJ)], axis=0)
        z_v[...] = a4.T

    def perhead_nn(w_v):
        def body(gi, acc):
            t0 = pl.multiple_of(gi * _TG, _TG)
            zg = z_v[pl.ds(t0, _TG), :]
            for s in range(_TG):
                lhs = jnp.where(dmask, zg[s:s + 1, :], 0.0).astype(BF16)
                rhs = w_v[:, t0 + s].reshape(NJ * H, D)
                acc = acc + jnp.dot(lhs, rhs, preferred_element_type=F32)
            return acc
        return lax.fori_loop(0, 128 // _TG, body, jnp.zeros((H, D), F32))

    def flash_step(off, carry):
        m, l, acc = carry
        ck = c_v[pl.ds(off, _TK), :]
        s = lax.dot_general(qa_v[...], ck, _NT, preferred_element_type=F32)
        m_new = jnp.maximum(m, jnp.max(s, axis=-1, keepdims=True))
        alpha = jnp.exp(m - m_new)
        p = jnp.exp(s - m_new)
        l = alpha * l + jnp.sum(p, axis=-1, keepdims=True)
        acc = alpha * acc + jnp.dot(p.astype(BF16), ck, preferred_element_type=F32)
        return m_new, l, acc

    carry = None
    for i, step in enumerate(order):
        kind = step[0]
        wait(i)
        if kind == "x":
            x = x_v[...].astype(F32)
            mean = jnp.mean(x, axis=-1, keepdims=True)
            xc = x - mean
            var = jnp.mean(xc * xc, axis=-1, keepdims=True)
            xn = (xc / jnp.sqrt(var + 1e-5)).astype(BF16).astype(F32)
            xf_v[0:16, :] = jnp.broadcast_to(x, (16, M))
            xf_v[16:32, :] = jnp.broadcast_to(xn, (16, M))
            prep_z(jnp.broadcast_to(xn, (H, M)))
        elif kind == "wq":
            q_v[...] = perhead_nn(wq_v).astype(BF16)
        elif kind == "wuk":
            def body(gi, carry_):
                t0 = pl.multiple_of(gi * _TG, _TG)
                q_b = q_v[...]
                rows = []
                for s in range(_TG):
                    rhs = wuk_v[:, t0 + s].reshape(NJ * H, D)
                    o = lax.dot_general(q_b, rhs, _NT, preferred_element_type=F32)
                    rows.append(jnp.sum(jnp.where(dmask, o, 0.0), axis=0, keepdims=True))
                y_v[pl.ds(t0, _TG), :] = jnp.concatenate(rows, axis=0)
                return carry_
            lax.fori_loop(0, 128 // _TG, body, 0)
            a4 = y_v[...].T
            q_abs = jnp.concatenate([a4[H * j:H * (j + 1), :] for j in range(NJ)], axis=1)
            qa_v[...] = (q_abs * (D ** -0.5)).astype(BF16)
            carry = (jnp.full((H, 1), -jnp.inf, F32), jnp.zeros((H, 1), F32), jnp.zeros((H, DC), F32))
        elif kind == "c":
            base, end = step[1], step[2]
            carry = lax.fori_loop(
                0, (end - base) // _TK,
                lambda k, cr, base=base: flash_step(pl.multiple_of(base + k * _TK, _TK), cr), carry)
            if end == SK:
                _, l, acc = carry
                prep_z((acc / l).astype(BF16).astype(F32))
        elif kind == "wuv":
            y_v[0:H, :] = perhead_nn(wuv_v)
            for h in range(H):
                l_v[:, h * D:(h + 1) * D] = jnp.broadcast_to(y_v[h:h + 1, :], (16, D)).astype(BF16)
            s_v[...] = jnp.zeros((16, M), F32)
            last = y_v[H - 1:H, :].astype(BF16).astype(F32)
            m_v[...] = jnp.broadcast_to(last, (D, D)).T
        elif kind == "wo":
            r0, r1 = step[1], step[2]
            s_new = s_v[...] + jnp.dot(l_v[:, r0:r1], wo_v[r0:r1, :], preferred_element_type=F32)
            if r1 == (H - 1) * D:
                s_new = xf_v[0:16, :] + s_new * g_v[...]
            s_v[...] = s_new
        elif kind == "wo_tail":
            r0, r1 = step[1], step[2]
            w = wo_v[r0:r1, :].astype(F32)
            mc = m_v[r0 - (H - 1) * D:r1 - (H - 1) * D, :]
            prod = w * jnp.concatenate([mc] * (M // 128), axis=1)
            part = prod[0:8, :]
            for k in range(1, (r1 - r0) // 8):
                part = part + prod[8 * k:8 * k + 8, :]
            if r0 > (H - 1) * D:
                part = p_v[...] + part
            if r1 < H * D:
                p_v[...] = part
            else:
                s_last = jnp.sum(part, axis=0, keepdims=True)
                o_v[...] = (s_v[0:1, :] + s_last * g_v[0:1, :]).astype(BF16)
        elif kind == "w1":
            xb = xf_v[16:32, :].astype(BF16)
            hpre = lax.dot_general(xb, w1_v[...], _NT, preferred_element_type=F32)
            hpre = hpre.astype(BF16).astype(F32)
            h_v[...] = (hpre * jax.nn.sigmoid(hpre)).astype(BF16)
        elif kind == "w2":
            gpre = jnp.dot(h_v[...], w2_v[...], preferred_element_type=F32)
            g_v[...] = gpre * jax.nn.sigmoid(gpre)

    cp_o = pltpu.make_async_copy(o_v, o_ref, sems.at[0])
    cp_o.start()
    cp_o.wait()


@jax.jit
def pallas_recurrent_scan__compressed_kv_cla__dense_activation_silu__decode_kernel(
    A_x: jax.Array,
    A_c_kv: jax.Array,
    A_w_q: jax.Array,
    A_w_uk: jax.Array,
    A_w_uv: jax.Array,
    A_w_o: jax.Array,
    B_x: jax.Array,
    B_w1: jax.Array,
    B_w2: jax.Array,
):
    del B_x
    _, SK, DC = A_c_kv.shape
    M, H, D = A_w_q.shape
    F = B_w1.shape[1]
    assert (M, DC, H, D) == (512, 512, 32, 128) and SK % (2 * _TK) == 0
    NJ = DC // 128

    half = SK // 2
    order = (
        ("x",), ("wq",), ("wuk",),
        ("c", 0, half), ("c", half, SK),
        ("w1",), ("w2",), ("wuv",),
        ("wo", 0, 22 * D), ("wo", 22 * D, 29 * D), ("wo", 29 * D, (H - 1) * D),
        ("wo_tail", (H - 1) * D, H * D - 32), ("wo_tail", H * D - 32, H * D),
    )

    def kernel(*refs):
        _kernel(order, SK, DC, H, D, M, F, *refs)

    out = pl.pallas_call(
        kernel,
        out_shape=jax.ShapeDtypeStruct((1, M), BF16),
        in_specs=[pl.BlockSpec(memory_space=pltpu.HBM)] * 8,
        out_specs=pl.BlockSpec(memory_space=pltpu.HBM),
        scratch_shapes=[
            pltpu.VMEM((1, M), BF16),
            pltpu.VMEM((SK, DC), BF16),
            pltpu.VMEM((NJ, 128, H, D), BF16),
            pltpu.VMEM((NJ, 128, H, D), BF16),
            pltpu.VMEM((NJ, 128, H, D), BF16),
            pltpu.VMEM((H * D, M), BF16),
            pltpu.VMEM((F, M), BF16),
            pltpu.VMEM((F, M), BF16),
            pltpu.VMEM((128, 128), F32),
            pltpu.VMEM((128, 128), F32),
            pltpu.VMEM((16, H * D), BF16),
            pltpu.VMEM((H, D), BF16),
            pltpu.VMEM((H, DC), BF16),
            pltpu.VMEM((16, F), BF16),
            pltpu.VMEM((16, M), F32),
            pltpu.VMEM((16, M), F32),
            pltpu.VMEM((32, M), F32),
            pltpu.VMEM((1, M), BF16),
            pltpu.VMEM((D, 128), F32),
            pltpu.VMEM((8, M), F32),
            pltpu.SemaphoreType.DMA((len(order),)),
        ],
        compiler_params=pltpu.CompilerParams(
            vmem_limit_bytes=100 * 1024 * 1024,
            disable_semaphore_checks=True,
        ),
    )(
        A_x.reshape(1, M),
        A_c_kv.reshape(SK, DC),
        A_w_q.reshape(NJ, 128, H, D),
        A_w_uk.reshape(NJ, 128, H, D),
        A_w_uv.reshape(NJ, 128, H, D),
        A_w_o.reshape(H * D, M),
        B_w1.T,
        B_w2,
    )
    return out.reshape(1, 1, M)
```

```python
import jax
import jax.numpy as jnp
from jax import lax
import jax.experimental.pallas as pl
import jax.experimental.pallas.tpu as pltpu

F32 = jnp.float32
BF16 = jnp.bfloat16
_NT = (((1,), (1,)), ((), ()))

_TK = 4096
_TG = 8
_WINDOW = 6


def _kernel(order, SK, DC, H, D, M, F,
            x_hbm, c_hbm, wq_hbm, wuk_hbm, wuv_hbm, wo_hbm, w1_hbm, w2_hbm, o_ref,
            x_v, c_v, wq_v, wuk_v, wuv_v, wo_v, w1_v, w2_v,
            z_v, y_v, l_v, q_v, qa_v, h_v, s_v, g_v, xf_v, o_v, m_v, p_v, sems):
    n = len(order)
    NJ = DC // 128

    def copy(i):
        step = order[i]
        kind, sem = step[0], sems.at[i]
        whole = {"x": (x_hbm, x_v), "wq": (wq_hbm, wq_v), "wuk": (wuk_hbm, wuk_v),
                 "wuv": (wuv_hbm, wuv_v), "w1": (w1_hbm, w1_v), "w2": (w2_hbm, w2_v)}
        if kind in whole:
            src, dst = whole[kind]
            return pltpu.make_async_copy(src, dst, sem)
        if kind == "c":
            src, dst, sl = c_hbm, c_v, pl.ds(step[1], step[2] - step[1])
        else:
            src, dst, sl = wo_hbm, wo_v, pl.ds(step[1], step[2] - step[1])
        return pltpu.make_async_copy(src.at[sl], dst.at[sl], sem)

    started = [0]

    def start_upto(k):
        while started[0] < min(k, n):
            copy(started[0]).start()
            started[0] += 1

    def wait(i):
        copy(i).wait()
        start_upto(i + 1 + _WINDOW)

    start_upto(_WINDOW)

    row = lax.broadcasted_iota(jnp.int32, (H, 128), 0)
    col = lax.broadcasted_iota(jnp.int32, (H, 128), 1)
    dmask = (col % H) == row

    def prep_z(a):
        a4 = jnp.concatenate([a[:, 128 * j:128 * (j + 1)] for j in range(NJ)], axis=0)
        z_v[...] = a4.T

    def perhead_nn(w_v):
        def body(gi, acc):
            t0 = pl.multiple_of(gi * _TG, _TG)
            zg = z_v[pl.ds(t0, _TG), :]
            for s in range(_TG):
                lhs = jnp.where(dmask, zg[s:s + 1, :], 0.0).astype(BF16)
                rhs = w_v[:, t0 + s].reshape(NJ * H, D)
                acc = acc + jnp.dot(lhs, rhs, preferred_element_type=F32)
            return acc
        return lax.fori_loop(0, 128 // _TG, body, jnp.zeros((H, D), F32))

    def flash_step(off, carry):
        m, l, acc = carry
        ck = c_v[pl.ds(off, _TK), :]
        s = lax.dot_general(qa_v[...], ck, _NT, preferred_element_type=F32)
        m_new = jnp.maximum(m, jnp.max(s, axis=-1, keepdims=True))
        alpha = jnp.exp(m - m_new)
        p = jnp.exp(s - m_new)
        l = alpha * l + jnp.sum(p, axis=-1, keepdims=True)
        acc = alpha * acc + jnp.dot(p.astype(BF16), ck, preferred_element_type=F32)
        return m_new, l, acc

    carry = None
    for i, step in enumerate(order):
        kind = step[0]
        wait(i)
        if kind == "x":
            x = x_v[...].astype(F32)
            mean = jnp.mean(x, axis=-1, keepdims=True)
            xc = x - mean
            var = jnp.mean(xc * xc, axis=-1, keepdims=True)
            xn = (xc / jnp.sqrt(var + 1e-5)).astype(BF16).astype(F32)
            xf_v[0:16, :] = jnp.broadcast_to(x, (16, M))
            xf_v[16:32, :] = jnp.broadcast_to(xn, (16, M))
            prep_z(jnp.broadcast_to(xn, (H, M)))
        elif kind == "wq":
            q_v[...] = perhead_nn(wq_v).astype(BF16)
        elif kind == "wuk":
            def body(gi, carry_):
                t0 = pl.multiple_of(gi * _TG, _TG)
                q_b = q_v[...]
                rows = []
                for s in range(_TG):
                    rhs = wuk_v[:, t0 + s].reshape(NJ * H, D)
                    o = lax.dot_general(q_b, rhs, _NT, preferred_element_type=F32)
                    rows.append(jnp.sum(jnp.where(dmask, o, 0.0), axis=0, keepdims=True))
                y_v[pl.ds(t0, _TG), :] = jnp.concatenate(rows, axis=0)
                return carry_
            lax.fori_loop(0, 128 // _TG, body, 0)
            a4 = y_v[...].T
            q_abs = jnp.concatenate([a4[H * j:H * (j + 1), :] for j in range(NJ)], axis=1)
            qa_v[...] = (q_abs * (D ** -0.5)).astype(BF16)
            carry = (jnp.full((H, 1), -jnp.inf, F32), jnp.zeros((H, 1), F32), jnp.zeros((H, DC), F32))
        elif kind == "c":
            base, end = step[1], step[2]
            carry = lax.fori_loop(
                0, (end - base) // _TK,
                lambda k, cr, base=base: flash_step(pl.multiple_of(base + k * _TK, _TK), cr), carry)
            if end == SK:
                _, l, acc = carry
                prep_z((acc / l).astype(BF16).astype(F32))
        elif kind == "wuv":
            y_v[0:H, :] = perhead_nn(wuv_v)
            for h in range(H):
                l_v[:, h * D:(h + 1) * D] = jnp.broadcast_to(y_v[h:h + 1, :], (16, D)).astype(BF16)
            s_v[...] = jnp.zeros((16, M), F32)
            last = y_v[H - 1:H, :].astype(BF16).astype(F32)
            m_v[...] = jnp.broadcast_to(last, (D, D)).T
        elif kind == "wo":
            r0, r1 = step[1], step[2]
            s_new = s_v[...] + jnp.dot(l_v[:, r0:r1], wo_v[r0:r1, :], preferred_element_type=F32)
            if r1 == (H - 1) * D:
                s_new = xf_v[0:16, :] + s_new * g_v[...]
            s_v[...] = s_new
        elif kind == "wo_tail":
            r0, r1 = step[1], step[2]
            w = wo_v[r0:r1, :].astype(F32)
            mc = m_v[r0 - (H - 1) * D:r1 - (H - 1) * D, :]
            prod = w * jnp.concatenate([mc] * (M // 128), axis=1)
            part = prod[0:8, :]
            for k in range(1, (r1 - r0) // 8):
                part = part + prod[8 * k:8 * k + 8, :]
            if r0 > (H - 1) * D:
                part = p_v[...] + part
            if r1 < H * D:
                p_v[...] = part
            else:
                s_last = jnp.sum(part, axis=0, keepdims=True)
                o_v[...] = (s_v[0:1, :] + s_last * g_v[0:1, :]).astype(BF16)
        elif kind == "w1":
            xb = xf_v[16:32, :].astype(BF16)
            hpre = lax.dot_general(xb, w1_v[...], _NT, preferred_element_type=F32)
            hpre = hpre.astype(BF16).astype(F32)
            h_v[...] = (hpre * jax.nn.sigmoid(hpre)).astype(BF16)
        elif kind == "w2":
            gpre = jnp.dot(h_v[...], w2_v[...], preferred_element_type=F32)
            g_v[...] = gpre * jax.nn.sigmoid(gpre)

    cp_o = pltpu.make_async_copy(o_v, o_ref, sems.at[0])
    cp_o.start()
    cp_o.wait()


@jax.jit
def pallas_recurrent_scan__compressed_kv_cla__dense_activation_silu__decode_kernel(
    A_x: jax.Array,
    A_c_kv: jax.Array,
    A_w_q: jax.Array,
    A_w_uk: jax.Array,
    A_w_uv: jax.Array,
    A_w_o: jax.Array,
    B_x: jax.Array,
    B_w1: jax.Array,
    B_w2: jax.Array,
):
    del B_x
    _, SK, DC = A_c_kv.shape
    M, H, D = A_w_q.shape
    F = B_w1.shape[1]
    assert (M, DC, H, D) == (512, 512, 32, 128) and SK % (2 * _TK) == 0
    NJ = DC // 128

    half = SK // 2
    order = (
        ("x",), ("wq",), ("wuk",),
        ("c", 0, half), ("c", half, SK),
        ("w1",), ("w2",), ("wuv",),
        ("wo", 0, 22 * D), ("wo", 22 * D, 29 * D), ("wo", 29 * D, (H - 1) * D),
        ("wo_tail", (H - 1) * D, H * D - 32), ("wo_tail", H * D - 32, H * D),
    )

    def kernel(*refs):
        pl.run_scoped(
            lambda sems: _kernel(order, SK, DC, H, D, M, F, *refs, sems),
            pltpu.SemaphoreType.DMA((len(order),)),
        )

    out = pl.pallas_call(
        kernel,
        out_shape=jax.ShapeDtypeStruct((1, M), BF16),
        in_specs=[pl.BlockSpec(memory_space=pltpu.HBM)] * 8,
        out_specs=pl.BlockSpec(memory_space=pltpu.HBM),
        scratch_shapes=[
            pltpu.VMEM((1, M), BF16),
            pltpu.VMEM((SK, DC), BF16),
            pltpu.VMEM((NJ, 128, H, D), BF16),
            pltpu.VMEM((NJ, 128, H, D), BF16),
            pltpu.VMEM((NJ, 128, H, D), BF16),
            pltpu.VMEM((H * D, M), BF16),
            pltpu.VMEM((F, M), BF16),
            pltpu.VMEM((F, M), BF16),
            pltpu.VMEM((128, 128), F32),
            pltpu.VMEM((128, 128), F32),
            pltpu.VMEM((16, H * D), BF16),
            pltpu.VMEM((H, D), BF16),
            pltpu.VMEM((H, DC), BF16),
            pltpu.VMEM((16, F), BF16),
            pltpu.VMEM((16, M), F32),
            pltpu.VMEM((16, M), F32),
            pltpu.VMEM((32, M), F32),
            pltpu.VMEM((1, M), BF16),
            pltpu.VMEM((D, 128), F32),
            pltpu.VMEM((8, M), F32),
        ],
        compiler_params=pltpu.CompilerParams(vmem_limit_bytes=100 * 1024 * 1024),
    )(
        A_x.reshape(1, M),
        A_c_kv.reshape(SK, DC),
        A_w_q.reshape(NJ, 128, H, D),
        A_w_uk.reshape(NJ, 128, H, D),
        A_w_uv.reshape(NJ, 128, H, D),
        A_w_o.reshape(H * D, M),
        B_w1.T,
        B_w2,
    )
    return out.reshape(1, 1, M)
```
